```python
import os as _os
_os.environ.setdefault("JAX_PLATFORMS", "cpu")
import jax
import jax.numpy as jnp

def _softmax(x, axis=-1):
    return jax.nn.softmax(x, axis=axis)
def _gelu(x):
    return jax.nn.gelu(x, approximate=True)
def _silu(x):
    return jax.nn.silu(x)
def _sigmoid(x):
    return jax.nn.sigmoid(x)
def _layernorm(x, axis=-1, eps=1e-5):
    m = jnp.mean(x, axis=axis, keepdims=True)
    v = jnp.var(x, axis=axis, keepdims=True)
    return (x - m) / jnp.sqrt(v + eps)
def _scatter_add(tgt, idx, src, axis=0):
    return tgt.at[idx].add(src)
def _segment_sum(src, seg, n):
    return jax.ops.segment_sum(src, seg, n)
class _Rng:
    def __init__(self, key):
        self._k = key
    def _next(self):
        self._k, sub = jax.random.split(self._k)
        return sub
    def normal(self, shape):
        return jax.random.normal(self._next(), shape, dtype=jnp.bfloat16)
    def randint(self, lo, hi, shape):
        return jax.random.randint(self._next(), shape, lo, hi, dtype=jnp.int32)
    def uniform(self, shape, lo=0.0, hi=1.0):
        return jax.random.uniform(self._next(), shape, jnp.bfloat16, lo, hi)
    def permutation(self, n):
        return jax.random.permutation(self._next(), n)


kernel_name = 'sequential_preLN__mha_block__moe_arch_mod__prompt'

def setup_inputs():
    _rng = _Rng(jax.random.key(int.from_bytes(__import__("os").urandom(4), "little")))
    _w = (lambda a: (lambda t: t.astype(jnp.bfloat16) if jnp.issubdtype(t.dtype, jnp.floating) else t)(jnp.asarray(a)))
    def _A_setup():
        B, S, D, H = 1, 2048, 640, 32
        return {
            "x": _w((lambda *s: _rng.normal(s) * 0.05)(B, S, D)),
            "wqkv": _w((lambda *s: _rng.normal(s) * 0.05)(D, 3 * D)),
            "wo": _w((lambda *s: _rng.normal(s) * 0.05)(D, D)),
        }
    _A_in = _A_setup()

    def _B_setup():
        B, S, D, F, C = 1, 2048, 640, 1536, 1
        return {
            "x": _w((lambda *s: _rng.normal(s) * 0.05)(B, S, D)),
            "w_r": _w((lambda *s: _rng.normal(s) * 0.05)(D)),
            "w_gate": _w((lambda *s: _rng.normal(s) * 0.05)(D, F)),
            "w_up": _w((lambda *s: _rng.normal(s) * 0.05)(D, F)),
            "w_down": _w((lambda *s: _rng.normal(s) * 0.05)(F, D)),
        }
    _B_in = _B_setup()

    return {
        "A_x": _A_in["x"],
        "A_wqkv": _A_in["wqkv"],
        "A_wo": _A_in["wo"],
        "B_x": _B_in["x"],
        "B_w_r": _B_in["w_r"],
        "B_w_gate": _B_in["w_gate"],
        "B_w_up": _B_in["w_up"],
        "B_w_down": _B_in["w_down"],
    }

def reference(A_x, A_wqkv, A_wo, B_x, B_w_r, B_w_gate, B_w_up, B_w_down):
    def _A_ref(x, wqkv, wo):
        B, S, D = x.shape
        H = 32
        Dh = D // H
        qkv = (lambda x, *d: x.transpose(*d))((x @ wqkv).reshape(B, S, 3, H, Dh), 2, 0, 3, 1, 4)
        q, k, v = qkv[0], qkv[1], qkv[2]
        scores = jnp.einsum("bhqd,bhkd->bhqk", q, k) * (Dh ** -0.5)
        p = _softmax(scores, axis=-1)
        o = jnp.einsum("bhqk,bhkd->bhqd", p, v)
        return (lambda x, *d: x.transpose(*d))(o, 0, 2, 1, 3).reshape(B, S, D) @ wo

    def _B_ref(x, w_r, w_gate, w_up, w_down):
        B, S, D = x.shape
        C = 1
        r = x @ w_r
        idx = jnp.argsort(-r, axis=-1)[:, :C]
        idx_e = jnp.repeat(idx.reshape(B, C, 1), D, axis=2)
        x_sel = jnp.take_along_axis(x, idx_e, axis=1)
        g = _silu(x_sel @ w_gate)
        u = x_sel @ w_up
        y = (g * u) @ w_down
        r_sel = _sigmoid(jnp.take_along_axis(r, idx, axis=1))
        y = y * r_sel.reshape(B, C, 1)
        b_off = (jnp.arange(B) * S).reshape(B, 1)
        flat_idx = (idx + b_off).reshape(B * C)
        zero = (x * 0.0).reshape(B * S, D)
        upd = _scatter_add(zero, flat_idx, y.reshape(B * C, D), axis=0)
        return x + upd.reshape(B, S, D)

    x = A_x
    h = x + _A_ref(_layernorm(x, axis=-1), A_wqkv, A_wo)
    h2 = h + _B_ref(_layernorm(h, axis=-1), B_w_r, B_w_gate, B_w_up, B_w_down)
    return h2
```

```python
import functools
import math
import jax
import jax.numpy as jnp
import jax.experimental.pallas as pl
import jax.experimental.pallas.tpu as pltpu

H = 32
DH = 20
HP = 32
EPS = 1e-5
LOG2E = math.log2(math.e)


def _ln(x):
    m = jnp.mean(x, axis=-1, keepdims=True)
    xc = x - m
    v = jnp.mean(xc * xc, axis=-1, keepdims=True)
    return xc * jax.lax.rsqrt(v + EPS)


def _kernel(x_ref, wqkv_ref, wo_ref, wr_ref, wg_hbm, wu_hbm, wd_hbm,
            out_ref,
            wt_s, wo_s, ln1_s, q_s, k_s, vt_s, ot_s, h_s, ln2_s, wg_ref, wu_ref, wd_ref, sems, *, qc):
    S, D = x_ref.shape
    DP = H * HP
    NT = (((1,), (1,)), ((), ()))
    TN = (((0,), (0,)), ((), ()))

    cps = [pltpu.make_async_copy(wg_hbm, wg_ref, sems.at[0]),
           pltpu.make_async_copy(wu_hbm, wu_ref, sems.at[1]),
           pltpu.make_async_copy(wd_hbm, wd_ref, sems.at[2])]
    for cp in cps:
        cp.start()

    zpad = jnp.zeros((HP - DH, D), jnp.float32)
    wt = wqkv_ref[...].astype(jnp.float32).T
    for i in range(3 * H):
        slab = jnp.concatenate([wt[i * DH:(i + 1) * DH, :], zpad], axis=0)
        wt_s[i * HP:(i + 1) * HP, :] = slab.astype(jnp.bfloat16)
    wo = wo_ref[...].astype(jnp.float32)
    for i in range(H):
        slab = jnp.concatenate([wo[i * DH:(i + 1) * DH, :], zpad], axis=0)
        wo_s[i * HP:(i + 1) * HP, :] = slab.astype(jnp.bfloat16)

    CH = 256
    for c in range(S // CH):
        xs = x_ref[c * CH:(c + 1) * CH, :].astype(jnp.float32)
        ln1_s[c * CH:(c + 1) * CH, :] = _ln(xs).astype(jnp.bfloat16)
    ln1 = ln1_s[...]
    q_s[...] = (jax.lax.dot_general(ln1, wt_s[0:DP, :], NT, preferred_element_type=jnp.float32)
                * (DH ** -0.5 * LOG2E)).astype(jnp.bfloat16)
    k_s[...] = jax.lax.dot_general(ln1, wt_s[DP:2 * DP, :], NT,
                                   preferred_element_type=jnp.float32).astype(jnp.bfloat16)
    vt = jax.lax.dot_general(wt_s[2 * DP:3 * DP, :], ln1, NT, preferred_element_type=jnp.float32)
    row = jax.lax.broadcasted_iota(jnp.int32, vt.shape, 0)
    vt = jnp.where((row & (HP - 1)) == DH, 1.0, vt)
    vt_s[...] = vt.astype(jnp.bfloat16)

    lane = jax.lax.broadcasted_iota(jnp.int32, (qc, 128), 1)
    nc = S // qc
    items = [(h, c) for h in range(H) for c in range(nc)]

    def scores(h, c):
        g, j = h // 4, h % 4
        kg = k_s[:, g * 128:(g + 1) * 128]
        qg = q_s[c * qc:(c + 1) * qc, g * 128:(g + 1) * 128]
        qm = jnp.where((lane >= j * HP) & (lane < (j + 1) * HP), qg, jnp.zeros_like(qg))
        return jax.lax.dot_general(kg, qm, NT, preferred_element_type=jnp.float32)

    def finish(h, c, st):
        m = jnp.max(st, axis=0, keepdims=True)
        pt = jnp.exp2(st - m).astype(jnp.bfloat16)
        ot = jnp.dot(vt_s[h * HP:(h + 1) * HP, :], pt, preferred_element_type=jnp.float32)
        ot = ot * pl.reciprocal(ot[DH:DH + 1, :], approx=False)
        ot_s[h * HP:(h + 1) * HP, c * qc:(c + 1) * qc] = ot.astype(jnp.bfloat16)

    s_next = scores(*items[0])
    for n, (h, c) in enumerate(items):
        st = s_next
        if n + 1 < len(items):
            s_next = scores(*items[n + 1])
        finish(h, c, st)

    attn = jax.lax.dot_general(ot_s[...], wo_s[...], TN, preferred_element_type=jnp.float32)
    attn = attn.astype(jnp.bfloat16)
    hh = (x_ref[...] + attn)
    hf = hh.astype(jnp.float32)
    ln2 = _ln(hf).astype(jnp.bfloat16)
    ln2f = ln2.astype(jnp.float32)
    h_s[...] = hf
    ln2_s[...] = ln2f
    out_ref[...] = hh + ln2
    r = jax.lax.dot_general(wr_ref[...], ln2, NT, preferred_element_type=jnp.float32)
    rr = r.astype(jnp.bfloat16).astype(jnp.float32)[0:1, :]

    rmax = jnp.max(rr)
    pos = jax.lax.broadcasted_iota(jnp.int32, rr.shape, 1)
    idx = jnp.min(jnp.where(rr == rmax, pos, S))
    base = pl.multiple_of((idx // 16) * 16, 16)
    rowm = jax.lax.broadcasted_iota(jnp.int32, (16, D), 0) == (idx - base)
    ln2_blk = ln2_s[pl.ds(base, 16), :]
    h_blk = h_s[pl.ds(base, 16), :]
    xsel = jnp.sum(jnp.where(rowm, ln2_blk, 0.0), axis=0, keepdims=True)
    xs8 = jnp.broadcast_to(xsel, (8, D)).astype(jnp.bfloat16)
    for cp in cps:
        cp.wait()
    gg = jnp.dot(xs8, wg_ref[...], preferred_element_type=jnp.float32).astype(jnp.bfloat16).astype(jnp.float32)
    gg = (gg * jax.nn.sigmoid(gg)).astype(jnp.bfloat16)
    uu = jnp.dot(xs8, wu_ref[...], preferred_element_type=jnp.float32).astype(jnp.bfloat16)
    y = jnp.dot(gg * uu, wd_ref[...], preferred_element_type=jnp.float32).astype(jnp.bfloat16)
    rs = jax.nn.sigmoid(rmax.astype(jnp.float32)).astype(jnp.bfloat16)
    y = (y * rs)[0:1, :]
    new = (h_blk.astype(jnp.bfloat16) + (ln2_blk.astype(jnp.bfloat16) + y))
    old = out_ref[pl.ds(base, 16), :]
    out_ref[pl.ds(base, 16), :] = jnp.where(rowm, new, old)


@jax.jit
def pallas_sequential_preLN__mha_block__moe_arch_mod__prompt_kernel(
    A_x: jax.Array,
    A_wqkv: jax.Array,
    A_wo: jax.Array,
    B_x: jax.Array,
    B_w_r: jax.Array,
    B_w_gate: jax.Array,
    B_w_up: jax.Array,
    B_w_down: jax.Array,
):
    tq = 2048
    B, S, D = A_x.shape
    F = B_w_gate.shape[1]
    x = A_x.reshape(S, D)
    wr = jnp.broadcast_to(B_w_r.reshape(1, D), (8, D))
    kern = functools.partial(_kernel, qc=tq)
    vm = pl.BlockSpec(memory_space=pltpu.VMEM)
    hbm = pl.BlockSpec(memory_space=pl.ANY)
    out = pl.pallas_call(
        kern,
        in_specs=[vm, vm, vm, vm, hbm, hbm, hbm],
        out_specs=vm,
        out_shape=jax.ShapeDtypeStruct((S, D), jnp.bfloat16),
        scratch_shapes=[
            pltpu.VMEM((3 * H * HP, D), jnp.bfloat16),
            pltpu.VMEM((H * HP, D), jnp.bfloat16),
            pltpu.VMEM((S, D), jnp.bfloat16),
            pltpu.VMEM((S, H * HP), jnp.bfloat16),
            pltpu.VMEM((S, H * HP), jnp.bfloat16),
            pltpu.VMEM((H * HP, S), jnp.bfloat16),
            pltpu.VMEM((H * HP, S), jnp.bfloat16),
            pltpu.VMEM((S, D), jnp.float32),
            pltpu.VMEM((S, D), jnp.float32),
            pltpu.VMEM((D, F), jnp.bfloat16),
            pltpu.VMEM((D, F), jnp.bfloat16),
            pltpu.VMEM((F, D), jnp.bfloat16),
            pltpu.SemaphoreType.DMA((3,)),
        ],
        compiler_params=pltpu.CompilerParams(vmem_limit_bytes=110 * 1024 * 1024),
    )(x, A_wqkv, A_wo, wr, B_w_gate, B_w_up, B_w_down)
    return out.reshape(B, S, D)
```

```python
import functools
import math
import jax
import jax.numpy as jnp
import jax.experimental.pallas as pl
import jax.experimental.pallas.tpu as pltpu

H = 32
DH = 20
HP = 32
HPG = 6
NG = (H + HPG - 1) // HPG
EPS = 1e-5
LOG2E = math.log2(math.e)


def _ln(x):
    m = jnp.mean(x, axis=-1, keepdims=True)
    xc = x - m
    v = jnp.mean(xc * xc, axis=-1, keepdims=True)
    return xc * jax.lax.rsqrt(v + EPS)


def _kernel(x_hbm, wqkv_hbm, wo_hbm, wr_ref, wg_hbm, wu_hbm, wd_hbm,
            out_ref,
            x_ref, wqkv_ref, wo_ref,
            wqk_s, wv_s, wo_s, ln1_s, q_s, k_s, vt_s, ot_s, h_s, ln2_s, wg_ref, wu_ref, wd_ref,
            s_buf, m_buf, p_buf, sems, *, qc, ur):
    S, D = x_ref.shape
    DP = H * HP
    DQ = NG * 128
    NT = (((1,), (1,)), ((), ()))
    TN = (((0,), (0,)), ((), ()))

    CH = 256
    NCH = S // CH
    cp_x = [pltpu.make_async_copy(x_hbm.at[c * CH:(c + 1) * CH, :], x_ref.at[c * CH:(c + 1) * CH, :],
                                  sems.at[6 + c]) for c in range(NCH)]
    cp_w = pltpu.make_async_copy(wqkv_hbm, wqkv_ref, sems.at[0])
    cp_o = pltpu.make_async_copy(wo_hbm, wo_ref, sems.at[2])
    cps = [pltpu.make_async_copy(wg_hbm, wg_ref, sems.at[3]),
           pltpu.make_async_copy(wu_hbm, wu_ref, sems.at[4]),
           pltpu.make_async_copy(wd_hbm, wd_ref, sems.at[5])]
    for cp in cp_x:
        cp.start()
    cp_w.start()
    cp_o.start()
    for cp in cps:
        cp.start()

    for c in range(NCH):
        cp_x[c].wait()
        xs = x_ref[c * CH:(c + 1) * CH, :].astype(jnp.float32)
        ln1_s[c * CH:(c + 1) * CH, :] = _ln(xs).astype(jnp.bfloat16)

    cp_w.wait()
    wt = wqkv_ref[...].astype(jnp.float32).T
    for t in range(2):
        for g in range(NG):
            nh = min(HPG, H - g * HPG)
            r0 = t * D + g * HPG * DH
            slab = jnp.concatenate([wt[r0:r0 + nh * DH, :],
                                    jnp.zeros((128 - nh * DH, D), jnp.float32)], axis=0)
            wqk_s[t * DQ + g * 128:t * DQ + (g + 1) * 128, :] = slab.astype(jnp.bfloat16)
    wv_s[...] = wt[2 * D:3 * D, :].astype(jnp.bfloat16)

    ln1 = ln1_s[...]
    vt = jax.lax.dot_general(wv_s[...], ln1, NT, preferred_element_type=jnp.float32)
    ones_pad = jnp.where(jax.lax.broadcasted_iota(jnp.int32, (HP - DH, S), 0) == 0, 1.0, 0.0)
    for h in range(H):
        slab = jnp.concatenate([vt[h * DH:(h + 1) * DH, :], ones_pad], axis=0)
        vt_s[h * HP:(h + 1) * HP, :] = slab.astype(jnp.bfloat16)
    q_s[...] = (jax.lax.dot_general(ln1, wqk_s[0:DQ, :], NT, preferred_element_type=jnp.float32)
                * (DH ** -0.5 * LOG2E)).astype(jnp.bfloat16)
    k_s[...] = jax.lax.dot_general(ln1, wqk_s[DQ:2 * DQ, :], NT,
                                   preferred_element_type=jnp.float32).astype(jnp.bfloat16)

    cp_o.wait()
    zpad = jnp.zeros((HP - DH, D), jnp.float32)
    wo = wo_ref[...].astype(jnp.float32)
    for i in range(H):
        slab = jnp.concatenate([wo[i * DH:(i + 1) * DH, :], zpad], axis=0)
        wo_s[i * HP:(i + 1) * HP, :] = slab.astype(jnp.bfloat16)

    lane = jax.lax.broadcasted_iota(jnp.int32, (qc, 128), 1)
    nc = S // qc
    N = H * nc

    def hc(n):
        return n // nc, n % nc

    def mo(v, m):
        return v if isinstance(v, int) else pl.multiple_of(v, m)

    def scores(n, slot):
        h, c = hc(n)
        g, j = h // HPG, h % HPG
        kg = k_s[:, pl.ds(mo(g * 128, 128), 128)]
        qg = q_s[pl.ds(mo(c * qc, qc), qc), pl.ds(mo(g * 128, 128), 128)]
        qm = jnp.where((lane >= j * DH) & (lane < (j + 1) * DH), qg, jnp.zeros_like(qg))
        st = jax.lax.dot_general(kg, qm, NT, preferred_element_type=jnp.float32)
        s_buf[slot] = st
        m_buf[slot] = jnp.broadcast_to(jnp.max(st, axis=0, keepdims=True), (8, qc))

    def softmax(n, slot):
        p_buf[slot] = jnp.exp2(s_buf[slot] - m_buf[slot][0:1, :]).astype(jnp.bfloat16)

    def pv(n, slot):
        h, c = hc(n)
        ot = jnp.dot(vt_s[pl.ds(mo(h * HP, HP), HP), :], p_buf[slot],
                     preferred_element_type=jnp.float32)
        ot = ot * pl.reciprocal(ot[DH:DH + 1, :], approx=False)
        ot_s[pl.ds(mo(h * HP, HP), HP), pl.ds(mo(c * qc, qc), qc)] = ot.astype(jnp.bfloat16)

    def step(nn, sl):
        scores(nn + 1, 1 - sl)
        softmax(nn, sl)
        pv(nn - 1, 1 - sl)

    scores(0, 0)
    scores(1, 1)
    softmax(0, 0)

    def body(n, carry):
        for u in range(ur):
            step(n * ur + 1 + u, (1 + u) % 2)
        return carry

    nit = (N - 2) // ur
    jax.lax.fori_loop(0, nit, body, 0)
    for nn in range(nit * ur + 1, N - 1):
        step(nn, nn % 2)
    softmax(N - 1, (N - 1) % 2)
    pv(N - 2, (N - 2) % 2)
    pv(N - 1, (N - 1) % 2)

    attn = jax.lax.dot_general(ot_s[...], wo_s[...], TN, preferred_element_type=jnp.float32)
    attn = attn.astype(jnp.bfloat16)
    hh = (x_ref[...] + attn)
    hf = hh.astype(jnp.float32)
    ln2 = _ln(hf).astype(jnp.bfloat16)
    ln2f = ln2.astype(jnp.float32)
    h_s[...] = hf
    ln2_s[...] = ln2f
    out_ref[...] = hh + ln2
    r = jax.lax.dot_general(wr_ref[...], ln2, NT, preferred_element_type=jnp.float32)
    rr = r.astype(jnp.bfloat16).astype(jnp.float32)[0:1, :]

    rmax = jnp.max(rr)
    pos = jax.lax.broadcasted_iota(jnp.int32, rr.shape, 1)
    idx = jnp.min(jnp.where(rr == rmax, pos, S - 1))
    base = pl.multiple_of((idx // 16) * 16, 16)
    rowm = jax.lax.broadcasted_iota(jnp.int32, (16, D), 0) == (idx - base)
    ln2_blk = ln2_s[pl.ds(base, 16), :]
    h_blk = h_s[pl.ds(base, 16), :]
    xsel = jnp.sum(jnp.where(rowm, ln2_blk, 0.0), axis=0, keepdims=True)
    xs8 = jnp.broadcast_to(xsel, (8, D)).astype(jnp.bfloat16)
    for cp in cps:
        cp.wait()
    gg = jnp.dot(xs8, wg_ref[...], preferred_element_type=jnp.float32).astype(jnp.bfloat16).astype(jnp.float32)
    gg = (gg * jax.nn.sigmoid(gg)).astype(jnp.bfloat16)
    uu = jnp.dot(xs8, wu_ref[...], preferred_element_type=jnp.float32).astype(jnp.bfloat16)
    y = jnp.dot(gg * uu, wd_ref[...], preferred_element_type=jnp.float32).astype(jnp.bfloat16)
    rs = jax.nn.sigmoid(rmax.astype(jnp.float32)).astype(jnp.bfloat16)
    y = (y * rs)[0:1, :]
    new = (h_blk.astype(jnp.bfloat16) + (ln2_blk.astype(jnp.bfloat16) + y))
    old = out_ref[pl.ds(base, 16), :]
    out_ref[pl.ds(base, 16), :] = jnp.where(rowm, new, old)


@jax.jit
def pallas_sequential_preLN__mha_block__moe_arch_mod__prompt_kernel(
    A_x: jax.Array,
    A_wqkv: jax.Array,
    A_wo: jax.Array,
    B_x: jax.Array,
    B_w_r: jax.Array,
    B_w_gate: jax.Array,
    B_w_up: jax.Array,
    B_w_down: jax.Array,
):
    tq, ur = 512, 12
    B, S, D = A_x.shape
    F = B_w_gate.shape[1]
    x = A_x.reshape(S, D)
    wr = jnp.broadcast_to(B_w_r.reshape(1, D), (8, D))
    kern = functools.partial(_kernel, qc=tq, ur=ur)
    vm = pl.BlockSpec(memory_space=pltpu.VMEM)
    hbm = pl.BlockSpec(memory_space=pl.ANY)
    DQ = NG * 128
    out = pl.pallas_call(
        kern,
        in_specs=[hbm, hbm, hbm, vm, hbm, hbm, hbm],
        out_specs=vm,
        out_shape=jax.ShapeDtypeStruct((S, D), jnp.bfloat16),
        scratch_shapes=[
            pltpu.VMEM((S, D), jnp.bfloat16),
            pltpu.VMEM((D, 3 * D), jnp.bfloat16),
            pltpu.VMEM((D, D), jnp.bfloat16),
            pltpu.VMEM((2 * DQ, D), jnp.bfloat16),
            pltpu.VMEM((D, D), jnp.bfloat16),
            pltpu.VMEM((H * HP, D), jnp.bfloat16),
            pltpu.VMEM((S, D), jnp.bfloat16),
            pltpu.VMEM((S, DQ), jnp.bfloat16),
            pltpu.VMEM((S, DQ), jnp.bfloat16),
            pltpu.VMEM((H * HP, S), jnp.bfloat16),
            pltpu.VMEM((H * HP, S), jnp.bfloat16),
            pltpu.VMEM((S, D), jnp.float32),
            pltpu.VMEM((S, D), jnp.float32),
            pltpu.VMEM((D, F), jnp.bfloat16),
            pltpu.VMEM((D, F), jnp.bfloat16),
            pltpu.VMEM((F, D), jnp.bfloat16),
            pltpu.VMEM((2, S, tq), jnp.float32),
            pltpu.VMEM((2, 8, tq), jnp.float32),
            pltpu.VMEM((2, S, tq), jnp.bfloat16),
            pltpu.SemaphoreType.DMA((14,)),
        ],
        compiler_params=pltpu.CompilerParams(vmem_limit_bytes=100 * 1024 * 1024),
    )(x, A_wqkv, A_wo, wr, B_w_gate, B_w_up, B_w_down)
    return out.reshape(B, S, D)
```
